```python
import os as _os
_os.environ.setdefault("JAX_PLATFORMS", "cpu")
import jax
import jax.numpy as jnp

def _softmax(x, axis=-1):
    return jax.nn.softmax(x, axis=axis)
def _gelu(x):
    return jax.nn.gelu(x, approximate=True)
def _silu(x):
    return jax.nn.silu(x)
def _sigmoid(x):
    return jax.nn.sigmoid(x)
def _layernorm(x, axis=-1, eps=1e-5):
    m = jnp.mean(x, axis=axis, keepdims=True)
    v = jnp.var(x, axis=axis, keepdims=True)
    return (x - m) / jnp.sqrt(v + eps)
def _scatter_add(tgt, idx, src, axis=0):
    return tgt.at[idx].add(src)
def _segment_sum(src, seg, n):
    return jax.ops.segment_sum(src, seg, n)
class _Rng:
    def __init__(self, key):
        self._k = key
    def _next(self):
        self._k, sub = jax.random.split(self._k)
        return sub
    def normal(self, shape):
        return jax.random.normal(self._next(), shape, dtype=jnp.bfloat16)
    def randint(self, lo, hi, shape):
        return jax.random.randint(self._next(), shape, lo, hi, dtype=jnp.int32)
    def uniform(self, shape, lo=0.0, hi=1.0):
        return jax.random.uniform(self._next(), shape, jnp.bfloat16, lo, hi)
    def permutation(self, n):
        return jax.random.permutation(self._next(), n)


kernel_name = 'standalone__gqa_block_cached__near_ridge'

def setup_inputs():
    _rng = _Rng(jax.random.key(int.from_bytes(__import__("os").urandom(4), "little")))
    _w = (lambda a: (lambda t: t.astype(jnp.bfloat16) if jnp.issubdtype(t.dtype, jnp.floating) else t)(jnp.asarray(a)))
    B, Sq, D = 16, 128, 576
    Hq, Hkv, Sk, Dh = 32, 16, 1024, 128
    assert Hq % Hkv == 0, (Hq, Hkv)
    return {
        "x": _w((lambda *s: _rng.normal(s) * 0.8)(B, Sq, D)),
        "k_cache": _w((lambda *s: _rng.normal(s) * 0.8)(B, Hkv, Sk, Dh)),
        "v_cache": _w((lambda *s: _rng.normal(s) * 0.05)(B, Hkv, Sk, Dh)),
        "wq": _w((lambda *s: _rng.normal(s) * 0.8)(D, Hq * Dh) * (D ** -0.5)),
        "wo": _w((lambda *s: _rng.normal(s) * 0.05)(Hq * Dh, D) * ((Hq * Dh) ** -0.5)),
    }

def reference(x, k_cache, v_cache, wq, wo):
    B, Sq, D = x.shape
    Hq, Dh = 32, 128
    Hkv = k_cache.shape[1]
    rep = Hq // Hkv
    q = (lambda x, *d: x.transpose(*d))((x @ wq).reshape(B, Sq, Hq, Dh), 0, 2, 1, 3)
    k = jnp.repeat(k_cache, rep, axis=1)
    v = jnp.repeat(v_cache, rep, axis=1)
    scores = jnp.einsum("bhqd,bhkd->bhqk", q, k) * (Dh ** -0.5)
    p = _softmax(scores, axis=-1)
    o = jnp.einsum("bhqk,bhkd->bhqd", p, v)
    return (lambda x, *d: x.transpose(*d))(o, 0, 2, 1, 3).reshape(B, Sq, Hq * Dh) @ wo
```

```python
import functools, math
import jax, jax.numpy as jnp
from jax import lax
import jax.experimental.pallas as pl
import jax.experimental.pallas.tpu as pltpu

NT = (((1,), (1,)), ((), ()))

def make(x, k_cache, v_cache, wq, wo, G=8, vmem=100, PCH=2, order=1, NS=2, only_loop=0, KC=1, rcp=1, late=0, nbc=1, LA=1):
    B, Sq, D = x.shape
    _, Hkv, Sk, Dh = k_cache.shape
    HD = wq.shape[1]
    rep = HD // Dh // Hkv
    nG = Hkv // G
    W = G * rep * Dh
    T = B * nG
    c = (Dh ** -0.5) * math.log2(math.e)
    xT = jnp.transpose(x, (0, 2, 1))
    woT = jnp.transpose(wo)
    nP = G // PCH
    WP = PCH * rep * Dh
    KS = Sk // KC
    bf = jnp.bfloat16

    def kern(x_hbm, k_hbm, v_hbm, wq_hbm, wo_hbm, o_hbm,
             xbuf, kvbuf, wq_ref, wo_ref, qbuf, obuf, acc_ref, out_buf,
             xsem, ksem, psem, wsem, osem):
        assert B & (B - 1) == 0
        LB = B.bit_length() - 1
        def gb(t):
            if isinstance(t, int): return t // B, t % B
            return lax.shift_right_logical(t, LB), t & (B - 1)
        def md(t, n):
            if isinstance(t, int): return t % n
            return t & (n - 1) if n & (n - 1) == 0 else lax.rem(t, n)
        def mul(a, n):
            return a * n if isinstance(a, int) else pl.multiple_of(a * n, n)
        def kcp(t):
            g, b = gb(t); s = md(t, NS)
            return pltpu.make_async_copy(k_hbm.at[b, pl.ds(g * G, G)], kvbuf.at[s, 0], ksem.at[s])
        def vcp(t):
            g, b = gb(t); s = md(t, NS)
            return pltpu.make_async_copy(v_hbm.at[b, pl.ds(g * G, G)], kvbuf.at[s, 1], ksem.at[s])
        def kcp0(j):
            return pltpu.make_async_copy(k_hbm.at[0, pl.ds(j * PCH, PCH)], kvbuf.at[0, 0, pl.ds(j * PCH, PCH)], psem.at[0, j])
        def vcp0(j):
            return pltpu.make_async_copy(v_hbm.at[0, pl.ds(j * PCH, PCH)], kvbuf.at[0, 1, pl.ds(j * PCH, PCH)], psem.at[1, j])
        def wqcp0(j):
            return pltpu.make_async_copy(wq_hbm.at[:, pl.ds(j * WP, WP)], wq_ref.at[:, pl.ds(j * WP, WP)], psem.at[2, j])
        def wqcp(g):
            return pltpu.make_async_copy(wq_hbm.at[:, pl.ds(mul(g, W), W)], wq_ref.at[:, pl.ds(mul(g, W), W)], wsem.at[0, g])
        def wocp(g):
            return pltpu.make_async_copy(wo_hbm.at[:, pl.ds(mul(g, W), W)], wo_ref.at[:, pl.ds(mul(g, W), W)], wsem.at[1, g])
        def xcp(b):
            return pltpu.make_async_copy(x_hbm.at[b], xbuf.at[b], xsem.at[b])
        def ocp(b):
            return pltpu.make_async_copy(out_buf.at[b], o_hbm.at[b], osem.at[b])
        def when(cond, fn):
            if isinstance(cond, bool):
                if cond: fn()
            else:
                pl.when(cond)(fn)

        def qproj(t):
            g, b = gb(t)
            q = jnp.dot(xbuf[b].T, wq_ref[:, pl.ds(mul(g, W), W)], preferred_element_type=jnp.float32)
            qbuf[md(t, 2)] = (q * c).astype(bf)

        def recip(l):
            if rcp == 0: return 1.0 / l
            r = pl.reciprocal(l, approx=True)
            return r * (2.0 - l * r)

        def attn_ops(getq, slot, heads, outs):
            st = {}
            qks, pvs = [], []
            for n, i in enumerate(heads):
                for kc in range(KC):
                    def qk(n=n, i=i, kc=kc):
                        if kc == 0:
                            st['q', n] = getq(n)
                        s = jax.lax.dot_general(st['q', n], kvbuf[slot, 0, i, kc * KS:(kc + 1) * KS], NT, preferred_element_type=jnp.float32)
                        mc = jnp.max(s, axis=1, keepdims=True)
                        if kc == 0:
                            m = mc; a = None
                        else:
                            m0 = st['m', n]
                            m = jnp.maximum(m0, mc)
                            a = jnp.exp2(m0 - m)
                        st['m', n] = m
                        p = jnp.exp2(s - m)
                        ls = jnp.sum(p, axis=1, keepdims=True)
                        st['l', n] = ls if kc == 0 else st['l', n] * a + ls
                        st['p', n, kc] = (p.astype(bf), a)
                    def pv(n=n, i=i, kc=kc):
                        p, a = st.pop(('p', n, kc))
                        o = jnp.dot(p, kvbuf[slot, 1, i, kc * KS:(kc + 1) * KS], preferred_element_type=jnp.float32)
                        if kc > 0: o = st['o', n] * a + o
                        st['o', n] = o
                        if kc == KC - 1:
                            o = (o * recip(st['l', n])).astype(bf)
                            outs.extend(o[r * Sq:(r + 1) * Sq] for r in range(rep))
                    qks.append(qk); pvs.append(pv)
            return qks, pvs

        def run_seq(qks, pvs, pre=(), mid=(), post=()):
            n = len(qks)
            la = min(LA, n)
            for j in range(la): qks[j]()
            for f in pre: f()
            for j in range(n):
                if j + la < n: qks[j + la]()
                if j == n - 1:
                    for f in mid: f()
                pvs[j]()
            for f in post: f()

        def q_from(q):
            return lambda n: jnp.concatenate([q[:, (n * rep + r) * Dh:(n * rep + r + 1) * Dh] for r in range(rep)], axis=0)

        def oproj(t):
            g, b = gb(t)
            y = jax.lax.dot_general(wo_ref[:, pl.ds(mul(g, W), W)], obuf[md(t, 2)], NT, preferred_element_type=jnp.float32)
            y = y + acc_ref[b]
            acc_ref[b] = y
            out_buf[b] = y.astype(bf)
            when(g == nG - 1, lambda: ocp(b).start())

        def step(t, last=False):
            g, b = gb(t)
            sl = md(t, NS)
            pltpu.make_async_copy(kvbuf.at[sl], kvbuf.at[sl], ksem.at[sl]).wait()
            if not last:
                def _ww():
                    wqcp(g + 1).wait(); wocp(g + 1).wait()
                when((b == B - 1) & (g < nG - 1), _ww)
                when(t < B - 1, lambda: xcp(t + 1).wait())
            def starts():
                if not last:
                    def _pf():
                        kcp(t + NS - 1).start(); vcp(t + NS - 1).start()
                    when(t + NS - 1 < T, _pf)
                    when(t < B - 2, lambda: xcp(t + 2).start())
                    def _w():
                        wqcp(g + 1).start(); wocp(g + 1).start()
                    when((b == 2) & (g < nG - 1), _w)
            if not late: starts()
            outs = []
            qks, pvs = attn_ops(q_from(qbuf[md(t, 2)]), sl, range(G), outs)
            def fin():
                obuf[md(t, 2)] = jnp.concatenate(outs, axis=1)
            op = [lambda: oproj(t - 1)]
            qp = [] if last else [lambda: qproj(t + 1)]
            if order == 0:   run_seq(qks, pvs, pre=op, mid=qp, post=[fin])
            elif order == 1: run_seq(qks, pvs, pre=op, post=[fin] + qp)
            elif order == 2: run_seq(qks, pvs, mid=op, post=[fin] + qp)
            elif order == 3: op[0](); run_seq(qks, pvs, mid=qp, post=[fin])
            elif order == 4: op[0](); run_seq(qks, pvs, post=[fin] + qp)
            elif order == 5: run_seq(qks, pvs, pre=qp, mid=op, post=[fin])
            if late: starts()

        def kv_drain(t):
            for tt in range(t, t + NS - 1):
                sl = tt % NS
                pltpu.make_async_copy(kvbuf.at[sl], kvbuf.at[sl], ksem.at[sl]).wait()
        def body(t, carry):
            step(t); return carry
        if only_loop:
            jax.lax.fori_loop(1, T - 1, body, 0)
            ocp(0).wait()
            return

        xcp(0).start()
        for j in range(nP):
            wqcp0(j).start(); kcp0(j).start(); vcp0(j).start()
        xcp(1).start()
        for s in range(1, NS):
            kcp(s).start(); vcp(s).start()
            if s == 1: wocp(0).start()
        xcp(2).start()
        acc_ref[...] = jnp.zeros(acc_ref.shape, acc_ref.dtype)
        xcp(0).wait()
        xb = xbuf[0].T
        outs = []
        for j in range(nP):
            wqcp0(j).wait()
            q = jnp.dot(xb, wq_ref[:, j * WP:(j + 1) * WP], preferred_element_type=jnp.float32)
            q = (q * c).astype(bf)
            kcp0(j).wait(); vcp0(j).wait()
            qks, pvs = attn_ops(q_from(q), 0, range(j * PCH, (j + 1) * PCH), outs)
            run_seq(qks, pvs)
        obuf[0] = jnp.concatenate(outs, axis=1)
        xcp(1).wait()
        qproj(1)
        wocp(0).wait()
        jax.lax.fori_loop(1, T - 1, body, 0)
        step(T - 1, last=True)
        oproj(T - 1)
        for b in range(B):
            ocp(b).wait()

    any_spec = pl.BlockSpec(memory_space=pltpu.HBM)
    outT = pl.pallas_call(
        kern,
        in_specs=[any_spec] * 5,
        out_specs=any_spec,
        out_shape=jax.ShapeDtypeStruct((B, D, Sq), x.dtype),
        scratch_shapes=[pltpu.VMEM((B, D, Sq), bf),
                        pltpu.VMEM((NS, 2, G, Sk, Dh), bf),
                        pltpu.VMEM((D, HD), bf), pltpu.VMEM((D, HD), bf),
                        pltpu.VMEM((2, Sq, W), bf), pltpu.VMEM((2, Sq, W), bf),
                        pltpu.VMEM((B, D, Sq), jnp.float32), pltpu.VMEM((B, D, Sq), bf),
                        pltpu.SemaphoreType.DMA((B,)), pltpu.SemaphoreType.DMA((NS,)),
                        pltpu.SemaphoreType.DMA((3, nP)), pltpu.SemaphoreType.DMA((2, nG)), pltpu.SemaphoreType.DMA((B,))],
        compiler_params=pltpu.CompilerParams(disable_bounds_checks=bool(nbc), vmem_limit_bytes=vmem * 1024 * 1024),
    )(xT, k_cache, v_cache, wq, woT)
    return jnp.transpose(outT, (0, 2, 1))


@jax.jit
def pallas_standalone__gqa_block_cached__near_ridge_kernel(x, k_cache, v_cache, wq, wo):
    return make(x, k_cache, v_cache, wq, wo, LA=2, KC=2, order=1, G=4)
```

```python
import math

import jax
import jax.numpy as jnp
from jax import lax
import jax.experimental.pallas as pl
import jax.experimental.pallas.tpu as pltpu

_NT = (((1,), (1,)), ((), ()))


def _gqa_block(x, k_cache, v_cache, wq, wo):
    B, Sq, D = x.shape
    _, Hkv, Sk, Dh = k_cache.shape
    HD = wq.shape[1]
    rep = HD // Dh // Hkv
    UH = 2
    UW = UH * rep * Dh
    nU = Hkv // UH
    segs = (3, 5)
    offs = (0, segs[0], nU)
    n0 = segs[0]
    P = 4
    LP = 2
    NF = P * n0
    KC = 2
    KS = Sk // KC
    OSPLIT = 2
    assert sum(segs) == nU and B >= P + 1 + (nU - n0) + 1 and 1 << LP == P
    assert Sk % (KC * 128) == 0 and D % (OSPLIT * 16) == 0
    qscale = (Dh ** -0.5) * math.log2(math.e)
    bf, f32 = jnp.bfloat16, jnp.float32

    def kern(x_hbm, k_hbm, v_hbm, wq_hbm, wo_hbm, o_hbm,
             xbuf, kvbuf, kvf, wq_ref, wo_ref, qc_ref, oc_ref, acc_ref, out_buf,
             xsem, kvsem, fsem, wsem, osem):

        def col(j):
            return pl.ds(j * UW if isinstance(j, int) else pl.multiple_of(j * UW, UW), UW)

        def kv_start(b, h0, n, dst, sem):
            pltpu.make_async_copy(k_hbm.at[b, pl.ds(h0, n)], dst(0), sem).start()
            pltpu.make_async_copy(v_hbm.at[b, pl.ds(h0, n)], dst(1), sem).start()

        def wait_all(buf, sem):
            pltpu.make_async_copy(buf, buf, sem).wait()

        def step_start(s, b, slot, u0=0, nu=None):
            nu = segs[s] if nu is None else nu
            lo = u0 * UH
            kv_start(b, offs[s] * UH + lo, nu * UH,
                     lambda w: kvbuf.at[slot, w, pl.ds(lo, nu * UH)], kvsem.at[slot])

        def fine_jb(k):
            return k >> LP, k & (P - 1)

        def fine_start(k):
            j, b = fine_jb(k)
            kv_start(b, j * UH, UH, lambda w: kvf.at[k, w], fsem.at[k])

        def wqcp(j):
            return pltpu.make_async_copy(wq_hbm.at[:, col(j)], wq_ref.at[:, col(j)], wsem.at[0, j])

        def wocp(j):
            return pltpu.make_async_copy(wo_hbm.at[:, col(j)], wo_ref.at[:, col(j)], wsem.at[1, j])

        def xcp(b):
            return pltpu.make_async_copy(x_hbm.at[b], xbuf.at[b], xsem.at[b])

        def ocp(b):
            return pltpu.make_async_copy(out_buf.at[b], o_hbm.at[b], osem.at[b])

        def qproj(xb, j):
            q = jnp.dot(xb, wq_ref[:, col(j)], preferred_element_type=f32)
            return (q * qscale).astype(bf)

        def oproj(o, b, j, final):
            R = D // OSPLIT
            for r in range(OSPLIT):
                rs = slice(r * R, (r + 1) * R)
                y = lax.dot_general(wo_ref[rs, col(j)], o, _NT, preferred_element_type=f32)
                y = y + acc_ref[b, rs]
                acc_ref[b, rs] = y
                if final:
                    out_buf[b, rs] = y.astype(out_buf.dtype)

        def recip(l):
            r = pl.reciprocal(l, approx=True)
            return r * (2.0 - l * r)

        class Attn:
            def __init__(self, kv):
                self.kv, self.st, self.q, self.o = kv, {}, {}, {}

            def qk(self, h, kc):
                st, qu, i = self.st, self.q[h // UH], h % UH
                q2 = jnp.concatenate(
                    [qu[:, (i * rep + r) * Dh:(i * rep + r + 1) * Dh] for r in range(rep)], axis=0)
                s = lax.dot_general(q2, self.kv[0, h, kc * KS:(kc + 1) * KS], _NT,
                                    preferred_element_type=f32)
                m = jnp.max(s, axis=1, keepdims=True)
                a = None
                if kc > 0:
                    m = jnp.maximum(st['m', h], m)
                    a = jnp.exp2(st['m', h] - m)
                st['m', h] = m
                p = jnp.exp2(s - m)
                ls = jnp.sum(p, axis=1, keepdims=True)
                st['l', h] = ls if kc == 0 else st['l', h] * a + ls
                st['p', h, kc] = (p.astype(bf), a)

            def pv(self, h, kc):
                st = self.st
                p, a = st.pop(('p', h, kc))
                o = jnp.dot(p, self.kv[1, h, kc * KS:(kc + 1) * KS], preferred_element_type=f32)
                if kc > 0:
                    o = st['o', h] * a + o
                st['o', h] = o
                if kc == KC - 1:
                    o = (o * recip(st['l', h])).astype(bf)
                    self.o.setdefault(h // UH, []).extend(o[r * Sq:(r + 1) * Sq] for r in range(rep))

            def unit_out(self, u):
                return jnp.concatenate(self.o.pop(u), axis=1)

        def compute(n, j0, b, kv, nxt, prv, final_prev):
            A = Attn(kv)
            A.q[0] = qc_ref[...]
            items = [(h, kc) for h in range(n * UH) for kc in range(KC)]
            ipu, ni = UH * KC, len(items)
            xb = xbuf[b].T if n > 1 else None
            if prv is not None:
                oproj(oc_ref[...], prv[0], prv[1], final_prev)
            A.qk(*items[0])
            if n > 1:
                A.q[1] = qproj(xb, j0 + 1)
            for i in range(ni):
                if i + 1 < ni:
                    A.qk(*items[i + 1])
                    u = (i + 1) // ipu
                    if (i + 1) % ipu == 0 and u + 1 < n:
                        A.q[u + 1] = qproj(xb, j0 + u + 1)
                A.pv(*items[i])
                d = i - 2
                if d >= 0 and d % ipu == ipu - 1 and d // ipu < n - 1:
                    oproj(A.unit_out(d // ipu), b, j0 + d // ipu, False)
            oc_ref[...] = A.unit_out(n - 1)
            qc_ref[...] = qproj(xbuf[nxt[0]].T, nxt[1])

        def fine_step(k):
            static = isinstance(k, int)
            when = (lambda c, fn: fn() if c else None) if static else (lambda c, fn: pl.when(c)(fn))
            j, b = fine_jb(k)
            wrap, end = b == P - 1, k == NF - 1
            wait_all(kvf.at[k], fsem.at[k])
            when(wrap & (k < NF - 1), lambda: wqcp(j + 1).wait())
            when(b == 1, lambda: wocp(j).wait())
            when(k < P - 1, lambda: xcp(k + 1).wait())
            when(end, lambda: xcp(P).wait())
            when(k + 2 < NF, lambda: fine_start(k + 2))
            when((k >= NF - 4) & (k < NF - 4 + n0),
                 lambda: step_start(0, P, P & 1, k - (NF - 4), 1))
            when((b == 0) & (j < n0 - 1), lambda: wqcp(j + 1).start())
            when((b == P - 2) & (j < n0 - 1), lambda: wocp(j + 1).start())
            when(k == NF - 4, lambda: xcp(P).start())
            when(k == NF - 2, lambda: xcp(P + 1).start())
            if static:
                nxt, prv = (b + 1, j), None
            else:
                nxt = (jnp.where(end, P, jnp.where(wrap, 0, b + 1)),
                       jnp.where(end, 0, jnp.where(wrap, j + 1, j)))
                prv = (jnp.where(b == 0, P - 1, b - 1), jnp.where(b == 0, j - 1, j))
            compute(1, j, b, kvf.at[k], nxt, prv, False)

        def make_body(s):
            first, last = s == 0, s == len(segs) - 1
            n = segs[s]

            def body(b, carry):
                slot = b & 1
                wait_all(kvbuf.at[slot, :, pl.ds(0, n * UH)], kvsem.at[slot])
                if first:
                    pl.when(b < B - 1)(lambda: xcp(b + 1).wait())

                    @pl.when(b == B - 1)
                    def _():
                        for j in range(n0, nU):
                            wqcp(j).wait()
                            wocp(j).wait()
                pl.when(b < B - 1)(lambda: step_start(s, b + 1, 1 - slot))
                if not last:
                    pl.when(b == B - 1)(lambda: step_start(s + 1, 0, 1 - slot))
                if first:
                    pl.when(b < B - 2)(lambda: xcp(b + 2).start())

                    @pl.when((b >= P + 1) & (b < P + 1 + nU - n0))
                    def _():
                        wqcp(n0 + b - P - 1).start()
                        wocp(n0 + b - P - 1).start()
                wrap_n, wrap_p = b == B - 1, b == 0
                nxt = (jnp.where(wrap_n, 0, b + 1), jnp.where(wrap_n, min(offs[s + 1], nU - 1), offs[s]))
                prv = (jnp.where(wrap_p, B - 1, b - 1),
                       jnp.where(wrap_p, max(offs[s] - 1, 0), offs[s + 1] - 1))
                compute(n, offs[s], b, kvbuf.at[slot], nxt, prv, last)
                if last:
                    pl.when(b > 0)(lambda: ocp(prv[0]).start())
                return carry
            return body

        xcp(0).start()
        wqcp(0).start()
        fine_start(0)
        acc_ref[...] = jnp.zeros(acc_ref.shape, f32)
        xcp(0).wait()
        wqcp(0).wait()
        for b in range(1, P):
            xcp(b).start()
        fine_start(1)
        wocp(0).start()
        qc_ref[...] = qproj(xbuf[0].T, 0)
        fine_step(0)

        def fine_body(k, carry):
            fine_step(k)
            return carry
        lax.fori_loop(1, NF, fine_body, 0)
        lax.fori_loop(P, B, make_body(0), 0)
        for s in range(1, len(segs)):
            lax.fori_loop(0, B, make_body(s), 0)
        oproj(oc_ref[...], B - 1, nU - 1, True)
        ocp(B - 1).start()
        for b in range(B):
            ocp(b).wait()

    assert B % 2 == 0 and P % 2 == 0
    hbm = pl.BlockSpec(memory_space=pltpu.HBM)
    outT = pl.pallas_call(
        kern,
        in_specs=[hbm] * 5,
        out_specs=hbm,
        out_shape=jax.ShapeDtypeStruct((B, D, Sq), x.dtype),
        scratch_shapes=[
            pltpu.VMEM((B, D, Sq), x.dtype),
            pltpu.VMEM((2, 2, max(segs) * UH, Sk, Dh), k_cache.dtype),
            pltpu.VMEM((NF, 2, UH, Sk, Dh), k_cache.dtype),
            pltpu.VMEM((D, HD), wq.dtype),
            pltpu.VMEM((D, HD), wo.dtype),
            pltpu.VMEM((Sq, UW), bf),
            pltpu.VMEM((Sq, UW), bf),
            pltpu.VMEM((B, D, Sq), f32),
            pltpu.VMEM((B, D, Sq), x.dtype),
            pltpu.SemaphoreType.DMA((B,)),
            pltpu.SemaphoreType.DMA((2,)),
            pltpu.SemaphoreType.DMA((NF,)),
            pltpu.SemaphoreType.DMA((2, nU)),
            pltpu.SemaphoreType.DMA((B,)),
        ],
        compiler_params=pltpu.CompilerParams(
            disable_bounds_checks=True, vmem_limit_bytes=100 * 1024 * 1024),
    )(jnp.transpose(x, (0, 2, 1)), k_cache, v_cache, wq, jnp.transpose(wo))
    return jnp.transpose(outT, (0, 2, 1))


@jax.jit
def pallas_standalone__gqa_block_cached__near_ridge_kernel(x, k_cache, v_cache, wq, wo):
    return _gqa_block(x, k_cache, v_cache, wq, wo)
```
